```python
import os as _os
_os.environ.setdefault("JAX_PLATFORMS", "cpu")
import jax
import jax.numpy as jnp

def _softmax(x, axis=-1):
    return jax.nn.softmax(x, axis=axis)
def _gelu(x):
    return jax.nn.gelu(x, approximate=True)
def _silu(x):
    return jax.nn.silu(x)
def _sigmoid(x):
    return jax.nn.sigmoid(x)
def _layernorm(x, axis=-1, eps=1e-5):
    m = jnp.mean(x, axis=axis, keepdims=True)
    v = jnp.var(x, axis=axis, keepdims=True)
    return (x - m) / jnp.sqrt(v + eps)
def _scatter_add(tgt, idx, src, axis=0):
    return tgt.at[idx].add(src)
def _segment_sum(src, seg, n):
    return jax.ops.segment_sum(src, seg, n)
class _Rng:
    def __init__(self, key):
        self._k = key
    def _next(self):
        self._k, sub = jax.random.split(self._k)
        return sub
    def normal(self, shape):
        return jax.random.normal(self._next(), shape, dtype=jnp.bfloat16)
    def randint(self, lo, hi, shape):
        return jax.random.randint(self._next(), shape, lo, hi, dtype=jnp.int32)
    def uniform(self, shape, lo=0.0, hi=1.0):
        return jax.random.uniform(self._next(), shape, jnp.bfloat16, lo, hi)
    def permutation(self, n):
        return jax.random.permutation(self._next(), n)


kernel_name = 'interleave_layers__spectral_gfnet__dense_activation_gelu__prompt'

def setup_inputs():
    _rng = _Rng(jax.random.key(int.from_bytes(__import__("os").urandom(4), "little")))
    _w = (lambda a: (lambda t: t.astype(jnp.bfloat16) if jnp.issubdtype(t.dtype, jnp.floating) else t)(jnp.asarray(a)))
    def _A_setup():
        B, S, D = 1, 2048, 640
        Df = D // 2 + 1
        return {
            "x": _w((lambda *s: _rng.normal(s) * 0.05)(B, S, D)),
            "w_r": _w((lambda *s: _rng.normal(s) * 0.2)(S, Df) * 0.02),
            "w_i": _w((lambda *s: _rng.normal(s) * 0.2)(S, Df) * 0.02),
        }
    _A_in = _A_setup()

    def _B_setup():
        B, S, D, F = 1, 2048, 640, 1728
        return {
            "x": _w((lambda *s: _rng.normal(s) * 0.05)(B, S, D)),
            "w1": _w((lambda *s: _rng.normal(s) * 0.1)(D, F) * (D ** -0.5)),
            "b1": _w((lambda *s: _rng.normal(s) * 0.1)(F) * 0.01),
            "w2": _w((lambda *s: _rng.normal(s) * 0.1)(F, D) * (F ** -0.5)),
            "b2": _w((lambda *s: _rng.normal(s) * 0.1)(D) * 0.01),
        }
    _B_in = _B_setup()

    return {
        "A_x": _A_in["x"],
        "A_w_r": _A_in["w_r"],
        "A_w_i": _A_in["w_i"],
        "B_x": _B_in["x"],
        "B_w1": _B_in["w1"],
        "B_b1": _B_in["b1"],
        "B_w2": _B_in["w2"],
        "B_b2": _B_in["b2"],
    }

def reference(A_x, A_w_r, A_w_i, B_x, B_w1, B_b1, B_w2, B_b2):
    def _A_ref(x, w_r, w_i):
        B, S, D = x.shape
        X = (lambda x, axes=(-2,-1): jnp.fft.rfft2(x.astype(jnp.float32), axes=axes))(x, axes=(-2, -1))
        W = w_r + 1j * w_i
        X = X * W
        y = (lambda x, s, axes=(-2,-1): jnp.fft.irfft2(x, s=s, axes=axes).astype(jnp.bfloat16))(X, (S, D), axes=(-2, -1))
        return y

    def _B_ref(x, w1, b1, w2, b2):
        h = jnp.einsum("bsd,df->bsf", x, w1) + b1
        h = _gelu(h)
        return jnp.einsum("bsf,fd->bsd", h, w2) + b2

    x = A_x
    x = x + _A_ref(_layernorm(x, axis=-1), A_w_r, A_w_i)
    x = x + _B_ref(_layernorm(x, axis=-1), B_w1, B_b1, B_w2, B_b2)
    x = x + _A_ref(_layernorm(x, axis=-1), A_w_r, A_w_i)
    x = x + _B_ref(_layernorm(x, axis=-1), B_w1, B_b1, B_w2, B_b2)
    return x
```

```python
import functools
import numpy as np
import jax, jax.numpy as jnp
from jax import lax
from jax.experimental import pallas as pl
from jax.experimental.pallas import tpu as pltpu

S, D, F, DF = 2048, 640, 1728, 321
NS, NL = 16, 128
NT = (((1,), (1,)), ((), ()))
f32, bf16, u32 = jnp.float32, jnp.bfloat16, jnp.uint32
p32 = lambda x: pltpu.bitcast(x, u32)
b16 = lambda x: pltpu.bitcast(x, bf16)
R2 = float(np.sqrt(0.5))
C1, C2 = float(np.cos(2 * np.pi / 5)), float(np.cos(4 * np.pi / 5))
S1, S2 = float(np.sin(2 * np.pi / 5)), float(np.sin(4 * np.pi / 5))
KQ = (C1 - C2) / 2

LA = np.concatenate([1 + 5 * np.arange(64), 4 + 5 * np.arange(64)])
LB = np.concatenate([2 + 5 * np.arange(64), 3 + 5 * np.arange(64)])
LH = 5 + 5 * np.arange(64)

def _consts():
    b = jnp.bfloat16
    d2 = np.arange(128)
    def fwd_mat(L, c, iscale):
        th = 2 * np.pi * ((np.outer(d2, L)) % D) / D
        sg = np.where(L % 5 == c, 1.0, -1.0)[None, :]
        top = np.concatenate([np.cos(th), -np.sin(th)], axis=1)
        bot = np.concatenate([sg * np.sin(th), sg * np.cos(th)], axis=1) * iscale
        return np.concatenate([top, bot], axis=0)
    MA = fwd_mat(LA, 1, -S1); MB = fwd_mat(LB, 2, -S2)
    th = 2 * np.pi * ((np.outer(d2, LH)) % D) / D
    MH = np.concatenate([np.cos(th), -np.sin(th)], axis=1)
    def inv_mat(L, c, iscale):
        th = 2 * np.pi * ((np.outer(L, d2)) % D) / D
        sg = np.where(L % 5 == c, 1.0, -1.0)[:, None]
        cw = 2.0 / (S * D)
        vr = np.concatenate([np.cos(th), -np.sin(th)], axis=0) * cw
        vi = np.concatenate([np.sin(th), np.cos(th)], axis=0) * np.concatenate([sg, sg], axis=0) * cw * iscale
        return np.concatenate([vr, vi], axis=1)
    NA = inv_mat(LA, 1, S1); NB = inv_mat(LB, 2, S1)
    th = 2 * np.pi * ((np.outer(LH, d2)) % D) / D
    cw = (np.where(LH == 320, 1.0, 2.0) / (S * D))[:, None]
    NH = np.concatenate([np.cos(th) * cw, -np.sin(th) * cw], axis=0)
    fm = np.zeros((256, 640)); fm[:, 0:256] = MA; fm[:, 256:512] = MB; fm[:128, 512:640] = MH
    im = np.zeros((256, 640)); im[:, 0:256] = NA; im[:, 256:512] = NB; im[:128, 512:640] = NH
    ka = np.arange(NS)[:, None, None]; kb = np.arange(NL)[None, :, None]; sl = np.arange(NL)[None, None, :]
    g = np.exp(-2j * np.pi * ((sl * (ka + NS * kb)) % S) / S)
    gf = np.concatenate([g.real, g.imag], axis=1)
    gh = np.conj(np.transpose(g, (0, 2, 1)))
    gi = np.concatenate([gh.real, gh.imag], axis=1)
    p = np.arange(NL); q = p % 16; base = p - q
    fcol = base + (q % 2) * 8 + q // 2
    gf = gf[:, :, fcol]
    irow = base + np.where(q < 8, 2 * q, 2 * (q - 8) + 1)
    gi = np.concatenate([gi[:, 0:128][:, irow], gi[:, 128:256][:, irow]], axis=1)
    def pk(a):
        a = np.asarray(a.astype(b)).view(np.uint16).astype(np.uint32)
        return a[..., 0::2, :] | (a[..., 1::2, :] << 16)
    return [pk(fm), pk(im), pk(gf), pk(gi)]

def layernorm(x):
    m = jnp.mean(x, axis=-1, keepdims=True)
    xc = x - m
    v = jnp.mean(xc * xc, axis=-1, keepdims=True)
    return xc * lax.rsqrt(v + 1e-5)

def gelu(h):
    c = float(np.sqrt(2 / np.pi))
    return (0.5 * h) * (1.0 + jnp.tanh(c * (h + 0.044715 * (h * h * h))))

def tiles(x):
    return [x[:, 128 * t:128 * (t + 1)] for t in range(x.shape[1] // 128)]

class Pair:
    def __init__(s, re, im): s.re, s.im = re, im
    def __add__(s, o): return Pair(s.re + o.re, s.im + o.im)
    def __sub__(s, o): return Pair(s.re - o.re, s.im - o.im)
    def add_i(s, o, sign):
        return Pair(s.re - o.im, s.im + o.re) if sign > 0 else Pair(s.re + o.im, s.im - o.re)
    def tw(s, num, sign):
        num = num % 16
        if num == 0: return s
        c = float(np.cos(2 * np.pi * num / 16)); sn = sign * float(np.sin(2 * np.pi * num / 16))
        if num % 4 == 0:
            q = num // 4
            if q == 2: return Pair(-s.re, -s.im)
            sg = sign if q == 1 else -sign
            return Pair(-s.im, s.re) if sg > 0 else Pair(s.im, -s.re)
        if num % 2 == 0:
            a = (s.re if c > 0 else -s.re); b = (s.im if c > 0 else -s.im)
            sg = 1.0 if sn * c > 0 else -1.0
            k = abs(c) * (1 if c > 0 else -1)
            if sg > 0:
                return Pair((s.re - s.im) * k, (s.re + s.im) * k)
            return Pair((s.re + s.im) * k, (s.im - s.re) * k)
        return Pair(s.re * c - s.im * sn, s.re * sn + s.im * c)

class Half:
    sgn = None
    def __init__(s, h): s.h = h
    def __add__(s, o): return Half(s.h + o.h)
    def __sub__(s, o): return Half(s.h - o.h)
    def add_i(s, o, sign):
        t = pltpu.roll(o.h, 64, 1) * Half.sgn
        return Half(s.h - t) if sign > 0 else Half(s.h + t)
    def tw(s, num, sign):
        num = num % 16
        if num == 0: return s
        c = float(np.cos(2 * np.pi * num / 16)); sn = sign * float(np.sin(2 * np.pi * num / 16))
        if num % 4 == 0:
            q = num // 4
            if q == 2: return Half(-s.h)
            sg = sign if q == 1 else -sign
            return Half(pltpu.roll(s.h, 64, 1) * (Half.sgn * (-sg)))
        return Half(s.h * c + pltpu.roll(s.h, 64, 1) * (Half.sgn * (-sn)))

def radix4(x, sign):
    a = x[0] + x[2]; b = x[0] - x[2]; c = x[1] + x[3]; d = x[1] - x[3]
    return [a + c, b.add_i(d, sign), a - c, b.add_i(d, -sign)]

def rdft8(b):
    t0 = b[0] + b[4]; t1 = b[0] - b[4]; t2 = b[2] + b[6]; t3 = b[2] - b[6]
    t4 = b[1] + b[5]; t5 = b[1] - b[5]; t6 = b[3] + b[7]; t7 = b[3] - b[7]
    s02 = t0 + t2; s46 = t4 + t6
    u = (t5 - t7) * R2; v = (t5 + t7) * R2
    C = [s02 + s46, t1 + u, t0 - t2, t1 - u, s02 - s46]
    Sn = [None, t3 + v, t4 - t6, v - t3, None]
    return C, Sn

def rdft16(a):
    Ec, Es = rdft8(a[0::2]); Oc, Os = rdft8(a[1::2])
    C = [None] * 9; Sn = [None] * 8
    C[0] = Ec[0] + Oc[0]; C[8] = Ec[0] - Oc[0]; C[4] = Ec[4]; Sn[4] = Oc[4]
    for k in (1, 2, 3):
        c = float(np.cos(2 * np.pi * k / 16)); s = float(np.sin(2 * np.pi * k / 16))
        if k == 2:
            P = (Oc[k] - Os[k]) * R2; Q = (Os[k] + Oc[k]) * R2
        else:
            P = c * Oc[k] - s * Os[k]; Q = c * Os[k] + s * Oc[k]
        C[k] = Ec[k] + P; C[8 - k] = Ec[k] - P
        Sn[k] = Es[k] + Q; Sn[8 - k] = Q - Es[k]
    return C, Sn

def dft16_half(a, sign, sgn_h):
    Ch, Sh = rdft16(a)
    out = [None] * 16
    out[0] = Ch[0]; out[8] = Ch[8]
    for k in range(1, 8):
        t = pltpu.roll(Sh[k], 64, 1) * sgn_h
        if sign < 0:
            out[k] = Ch[k] + t; out[16 - k] = Ch[k] - t
        else:
            out[k] = Ch[k] - t; out[16 - k] = Ch[k] + t
    return out

def make(stop=99, plan=0, wmix=True, dmaorder=0, flags=None, only=None, nch=8, prog=0):
    CH = 16
    NCH = NL // CH
    RC = NS * CH
    consts = _consts()
    W4 = lambda j: ' '.join(f'W{i}' for i in range(4 * j, 4 * j + 4))
    R0PROG = [
        ">fd >x0 >x1 ?fd ?x0 >x2 >x3 >x4 >x5 >x6 >x7 X0 | ?x1 B0 X1 | ?x2 >w0 B1 X2 C0 | ?x3 >w1 B2 X3 C1 | ?x4 >w2 B3 X4 C2 | ?x5 >w3 >g0 B4 X5 C3 | "
        f"?x6 ?w0 >g1 B5 X6 C4 {W4(0)} | ?x7 ?w1 >g2 B6 X7 C5 {W4(1)} | ?w2 >g3 >fi B7 C6 {W4(2)} | ?w3 >m1 >m2 C7 {W4(3)}",
        ">fd >x0 >x1 ?fd ?x0 >x2 >x3 >x4 >x5 >x6 >x7 X0 | ?x1 ?x2 >w0 B0 X1 B1 X2 C0 | ?x3 ?x4 >w1 >w2 B2 X3 C1 B3 X4 C2 | ?x5 ?x6 ?x7 ?w0 >w3 >g0 >g1 B4 X5 C3 B5 X6 C4 "
        f"{W4(0)} | ?w1 ?w2 >g2 >g3 >fi B6 X7 C5 {W4(1)} B7 C6 {W4(2)} | ?w3 >m1 >m2 C7 {W4(3)}",
        ">fd >x0 >x1 ?fd ?x0 >x2 >x3 >x4 >x5 >x6 >x7 X0 | ?x1 ?x2 ?x3 >w0 >w1 B0 X1 B1 X2 C0 B2 X3 C1 | ?x4 ?x5 ?x6 ?x7 >w2 >w3 >g0 >g1 B3 X4 C2 B4 X5 C3 B5 X6 C4 B6 X7 C5 | "
        f"?w0 ?w1 >g2 >g3 >fi B7 C6 {W4(0)} {W4(1)} | ?w2 ?w3 >m1 >m2 C7 {W4(2)} {W4(3)}",
        ">fd >x0 >x1 ?fd ?x0 >x2 >x3 >x4 >x5 >x6 >x7 X0 | ?x1 ?x2 ?x3 >w0 >w1 B0 X1 B1 X2 C0 B2 X3 C1 | ?x4 ?x5 ?x6 ?x7 ?w0 >w2 >w3 >g0 >g1 B3 X4 C2 B4 X5 C3 W0 W1 B5 X6 C4 W2 W3 | "
        f"?w1 ?w2 >g2 >g3 >fi B6 X7 C5 {W4(1)} B7 C6 {W4(2)} | ?w3 >m1 >m2 C7 {W4(3)}",
    ][prog]
    DSCHED = [
        {0: ['w0'], 2: ['w1'], 4: ['w2'], 5: ['g0'], 6: ['w3'], 8: ['g1'], 9: ['fi', 'm1', 'm2']},
        {1: ['w0', 'w1', 'w2', 'w3'], 3: ['g0'], 4: ['g1', 'fi'], 6: ['m1', 'm2']},
        {2: ['w0', 'w1', 'w2', 'w3'], 4: ['g0', 'g1', 'fi'], 7: ['m1'], 9: ['m2']},
        {1: ['w0', 'w1'], 2: ['w2', 'w3'], 4: ['g0', 'g1', 'fi'], 7: ['m1'], 8: ['m2']},
        {0: ['w0'], 1: ['w1'], 2: ['w2'], 3: ['w3'], 4: ['g0'], 5: ['g1', 'fi'], 7: ['m1'], 9: ['m2']},
    ][dmaorder]

    def kern(x_hbm, wrt_hbm, wit_hbm, w1t_hbm, b1_ref, w2_hbm, b2_ref, fd_hbm, fi_hbm, gf_hbm, gi_hbm,
             o_hbm,
             xbuf, res, wrt, wit, wtf, w1t, w2, fd, fi, gf, gi, wp, ubuf, vbuf, obuf,
             xnb, gbuf, ub, abuf, tbuf, zbuf, abuf2, tbuf2, sem_x, sem_w, sem_o, sem_g, sem_m):
        xcopies = [pltpu.make_async_copy(x_hbm.at[:, c], xbuf.at[c], sem_x.at[c]) for c in range(NCH)]
        WJ = 4
        NWP = 16 // WJ
        wsl = lambda j: pl.ds(j * WJ * 128, WJ * 128)
        wpieces = [[pltpu.make_async_copy(h.at[:, wsl(j)], v.at[:, wsl(j)], sem_w.at[2 * j + i]) for i, (h, v) in enumerate(((wrt_hbm, wrt), (wit_hbm, wit)))] for j in range(NWP)]
        GP = 4
        gpieces = [[pltpu.make_async_copy(h.at[pl.ds(j * GP, GP)], v.at[pl.ds(j * GP, GP)], sem_g.at[2 * j + i]) for i, (h, v) in enumerate(((gf_hbm, gf), (gi_hbm, gi)))] for j in range(NS // GP)]
        fd_cp = pltpu.make_async_copy(fd_hbm, fd, sem_m.at[0])
        fi_cp = pltpu.make_async_copy(fi_hbm, fi, sem_m.at[1])
        w1_cp = pltpu.make_async_copy(w1t_hbm, w1t, sem_m.at[2])
        w2_cp = pltpu.make_async_copy(w2_hbm, w2, sem_m.at[3])
        def start(l):
            for c_ in l: c_.start()
        def wait(l):
            for c_ in l: c_.wait()

        lane = lax.broadcasted_iota(jnp.int32, (1, 128), 1)
        sgn_h = jnp.where(lane < 64, 1.0, -1.0).astype(f32)
        Half.sgn = sgn_h

        def rs(s, n=CH):
            return pl.ds(n * s, n)

        GRP = [(0, 1), (2, 3), (4,)]
        GO = (2, 0, 1)
        def ld(ref, idx, grp):
            if len(grp) == 2:
                return Pair(ref[idx + (pl.ds(128 * grp[0], 128),)], ref[idx + (pl.ds(128 * grp[1], 128),)])
            return Half(ref[idx + (pl.ds(128 * grp[0], 128),)])
        def st(ref, idx, grp, val, dt=None):
            cv = (lambda a: pltpu.pack_elementwise([a[0:8], a[8:16]], packed_dtype=bf16)) if dt is not None else (lambda a: a)
            if len(grp) == 2:
                ref[idx + (pl.ds(128 * grp[0], 128),)] = cv(val.re)
                ref[idx + (pl.ds(128 * grp[1], 128),)] = cv(val.im)
            else:
                ref[idx + (pl.ds(128 * grp[0], 128),)] = cv(val.h)

        def A_piece(c, r0, nr, src=None):
            x = res[c, pl.ds(r0, nr), :] if src is None else src
            xn = layernorm(x)
            x0, x1, x2, x3, x4 = tiles(xn)
            t1 = x1 + x4; t2 = x2 + x3; t3 = x1 - x4; t4 = x2 - x3
            p = t1 + t2; q = (t1 - t2) * KQ
            u0 = x0 + p; m = x0 - 0.25 * p
            u1r = m + q; u2r = m - q
            u1i = t3 + (S2 / S1) * t4; u2i = t3 - (S1 / S2) * t4
            ub[pl.ds((c % 2) * (RC // 2) + r0 // 2, nr // 2), :] = p32(jnp.concatenate([u1r, u1i, u2r, u2i, u0], axis=1).astype(bf16))

        def B_piece(c, g, ab=None):
            ab = abuf if ab is None else ab
            lo = (0, 256, 512)[g]; w = (256, 256, 128)[g]
            ab[:, lo:lo + w] = jnp.dot(b16(ub[pl.ds((c % 2) * (RC // 2), RC // 2), lo:lo + w]), b16(fd[0:w // 2, lo:lo + w]), preferred_element_type=f32)

        def C1_piece(g, s0, ab=None):
            ab = abuf if ab is None else ab
            grp = GRP[g]
            x = [ld(ab, (rs(4 * s1 + s0),), grp) for s1 in range(4)]
            y = radix4(x, -1)
            for k1 in range(4):
                st(tbuf, (rs(4 * s0 + k1),), grp, y[k1].tw(k1 * s0, -1))

        def C2_piece(c, g, k1):
            grp = GRP[g]
            x = [ld(tbuf, (rs(4 * s0 + k1),), grp) for s0 in range(4)]
            y = radix4(x, -1)
            for k2 in range(4):
                st(ubuf, (pl.ds((k1 + 4 * k2) * (NL // 2) + c * CH // 2, CH // 2),), grp, y[k2], bf16)

        def CH_piece(c, ab=None):
            ab = abuf if ab is None else ab
            x = [ab[rs(s_), 512:640] for s_ in range(NS)]
            y = dft16_half(x, -1, sgn_h)
            for k in range(NS):
                ubuf[pl.ds(k * (NL // 2) + c * CH // 2, CH // 2), 512:640] = pltpu.pack_elementwise([y[k][0:8], y[k][8:16]], packed_dtype=bf16)

        def DH_piece(c):
            x = [vbuf[k, pl.ds(c * CH, CH), 512:640] for k in range(NS)]
            y = dft16_half(x, 1, sgn_h)
            for s_ in range(NS):
                zbuf[rs(s_, CH // 2), 512:640] = pltpu.pack_elementwise([y[s_][0:8], y[s_][8:16]], packed_dtype=bf16)

        def D1_piece(c, g, k0):
            grp = GRP[g]
            x = [ld(vbuf, (4 * k1 + k0, pl.ds(c * CH, CH)), grp) for k1 in range(4)]
            y = radix4(x, 1)
            for s1 in range(4):
                st(tbuf2, (rs(4 * k0 + s1),), grp, y[s1].tw(s1 * k0, 1))

        def D2_piece(g, s1):
            grp = GRP[g]
            x = [ld(tbuf2, (rs(4 * k0 + s1),), grp) for k0 in range(4)]
            y = radix4(x, 1)
            for s2 in range(4):
                st(zbuf, (rs(s1 + 4 * s2, CH // 2),), grp, y[s2], bf16)

        def E_piece(g):
            lo = (0, 256, 512)[g]; w = (256, 256, 128)[g]
            abuf2[:, lo:lo + w] = jnp.dot(b16(zbuf[:, lo:lo + w]), b16(fi[0:w // 2, lo:lo + w]), preferred_element_type=f32)

        def E2_piece(c, r0, nr, slot, first=False):
            v1r, a1, v2r, a2, v0 = tiles(abuf2[pl.ds(r0, nr), :])
            t1 = v1r + v2r; n = (v1r - v2r) * KQ
            y0 = v0 + t1; m = v0 - 0.25 * t1
            aa = m + n; bb = m - n
            p = a1 + (S2 / S1) * a2; q = (S2 / S1) * a1 - a2
            y = jnp.concatenate([y0, aa - p, bb - q, bb + q, aa + p], axis=1)
            x0_ = xbuf[c].reshape(RC, D).astype(f32) if first else res[c]
            x1 = x0_ + y
            res[c, pl.ds(r0, nr), :] = x1
            if slot is not None:
                xnb[pl.ds(slot * (RC // 2) + r0 // 2, nr // 2), :] = p32(layernorm(x1).astype(bf16))

        b1v = lambda a, b: b1_ref[...].astype(f32).reshape(1, F)[:, a:b]
        b2v = lambda a, b: b2_ref[...].astype(f32).reshape(1, D)[:, a:b]
        M1E = [0, 256, 512, 768, 1024, 1280, 1536, F]
        def M1_piece(slot, j):
            a, b = M1E[j], M1E[j + 1]
            h = lax.dot_general(b16(xnb[pl.ds(slot * (RC // 2), RC // 2), :]), w1t[a:b, :], NT, preferred_element_type=f32) + b1v(a, b)
            gbuf[:, a:b] = p32(gelu(h).astype(bf16))

        def M2_piece(c, t, last):
            a, b = 128 * t, 128 * (t + 1)
            o = jnp.dot(b16(gbuf[...]), w2[:, a:b], preferred_element_type=f32) + b2v(a, b)
            x2 = res[c, :, a:b] + o
            if last:
                obuf[c, :, :, a:b] = x2.astype(bf16).reshape(NS, CH, 128)
            else:
                res[c, :, a:b] = x2

        def out_start(c):
            pltpu.make_async_copy(obuf.at[c], o_hbm.at[:, c], sem_o.at[c]).start()

        rr = lax.broadcasted_iota(jnp.int32, (128, 128), 0)
        cc = lax.broadcasted_iota(jnp.int32, (128, 128), 1)
        pm = jnp.where((rr // 8) + 16 * (rr % 8) == cc, 1.0, 0.0).astype(bf16)

        def wfix(j):
            wtf[0, j] = wrt[:, 128 * j:128 * (j + 1)].astype(f32)
            wtf[1, j] = wit[:, 128 * j:128 * (j + 1)].astype(f32)

        def wprep(j):
            r8 = j * 8
            def g(i, c0, c1):
                return jnp.concatenate([wtf[i, j, pl.ds(c0, 64, stride=5), :], wtf[i, j, pl.ds(c1, 64, stride=5), :]], axis=0).astype(bf16)
            rhs = [g(0, 1, 4), g(1, 1, 4), g(0, 2, 3), g(1, 2, 3), g(0, 5, 5), g(1, 5, 5)]
            outs = [lax.dot_general(pm, r, NT, preferred_element_type=f32) for r in rhs]
            outs[5] = outs[5] * (-sgn_h)
            for t in range(6):
                for ka in range(NS):
                    wp[ka, pl.ds(r8, 8), 128 * t:128 * (t + 1)] = outs[t][8 * ka:8 * (ka + 1)]

        def cmul_combine(p):
            p1 = tiles(p[0:128]); p2 = tiles(p[128:256])
            return [p1[0] - p2[1], p1[1] + p2[0], p1[2] - p2[3], p1[3] + p2[2],
                    p1[4] - pltpu.roll(p2[4], 64, 1) * sgn_h]

        def col_a(ka):
            return jnp.dot(b16(gf[ka]), b16(ubuf[pl.ds(ka * (NL // 2), NL // 2), :]), preferred_element_type=f32)

        def col_b(ka, p):
            xq = cmul_combine(p)
            w = tiles(wp[ka])
            y = [xq[0] * w[0] - xq[1] * w[1], xq[0] * w[1] + xq[1] * w[0],
                 xq[2] * w[2] - xq[3] * w[3], xq[2] * w[3] + xq[3] * w[2],
                 xq[4] * w[4] + pltpu.roll(xq[4], 64, 1) * w[5]]
            return jnp.concatenate(y, axis=1).astype(bf16)

        def col_c(ka, yb):
            q2 = jnp.dot(b16(gi[ka]), yb, preferred_element_type=f32)
            vbuf[ka] = jnp.concatenate(cmul_combine(q2), axis=1)

        def conv_w(src, dst, i, n):
            r0 = i * (F // 2 // n) ; nr = F // 2 // n
            dst[pl.ds(r0, nr), :] = p32(src[pl.ds(2 * r0, 2 * nr), :])

        def col_phase(first):
            if first: wait(gpieces[0]); wait(gpieces[1])
            p = col_a(0)
            for ka in range(NS):
                if first and ka + 1 == 8: wait(gpieces[2]); wait(gpieces[3])
                pn = col_a(ka + 1) if ka + 1 < NS else None
                col_c(ka, col_b(ka, p))
                p = pn

        def fwd_all(c, src_rows=None):
            A_piece(c, 0, RC)
            for g in GO: B_piece(c, g)
            CH_piece(c)
            for g in (0, 1):
                for s0 in range(4): C1_piece(g, s0)
                for k1 in range(4): C2_piece(c, g, k1)

        def inv_all(c, slot, first=False):
            DH_piece(c)
            for g in (0, 1):
                for k0 in range(4): D1_piece(c, g, k0)
                for s1 in range(4): D2_piece(g, s1)
            for g in GO: E_piece(g)
            E2_piece(c, 0, RC, slot, first)

        def row_phase(last):
            conv2 = (not last) and only is None
            inv_all(0, 0, not last)
            for c in range(nch):
                sl = c % 2
                side = {i: [] for i in range(12)}
                doA = (not last) and c > 0
                doD = c + 1 < NCH
                P = lambda f, *a: (lambda: f(*a))
                Cp = lambda g: [P(CH_piece, c - 1)] if g == 2 else [P(C1_piece, g, s0) for s0 in range(4)] + [P(C2_piece, c - 1, g, k1) for k1 in range(4)]
                Dp = lambda g: [P(DH_piece, c + 1)] if g == 2 else [P(D1_piece, c + 1, g, k0) for k0 in range(4)] + [P(D2_piece, g, s1) for s1 in range(4)]
                Ap = P(A_piece, c - 1, 0, RC)
                Bp = lambda g: P(B_piece, c - 1, g)
                Ep = lambda g: P(E_piece, g)
                E2p = P(E2_piece, c + 1, 0, RC, 1 - sl, not last)
                def spread(lst, slots):
                    n = len(slots)
                    for i, sl_ in enumerate(slots):
                        side[sl_] += lst[len(lst) * i // n:len(lst) * (i + 1) // n]
                if plan == 0:
                    if doA:
                        side[0] += [Ap]
                        side[1] += [Bp(g) for g in GO]
                        spread(Cp(2) + Cp(0) + Cp(1), [2, 3, 4])
                    if doD:
                        spread(Dp(2) + Dp(0) + Dp(1), [5, 6, 7])
                        side[8] += [Ep(g) for g in GO]
                        side[9] += [E2p]
                elif plan == 1:
                    if doA:
                        side[0] += [Ap]
                        for i_, g in enumerate(GO):
                            side[7 + i_] += [Bp(g)]
                            side[8 + i_] += Cp(g)
                    if doD:
                        spread(Dp(2) + Dp(0) + Dp(1), [2, 3, 4, 5, 6])
                        side[6] += [Ep(g) for g in GO]
                        side[7] = [E2p] + side[7]
                elif plan == 2:
                    if doA:
                        side[0] += [Ap]
                        for i_, g in enumerate(GO):
                            side[2 + 2 * i_] += [Bp(g)]
                            side[3 + 2 * i_] += Cp(g)
                    if doD:
                        spread(Dp(2) + Dp(0) + Dp(1), [7, 8])
                        side[8] += [Ep(g) for g in GO]
                        side[9] += [E2p]
                elif plan == 4:
                    if doA:
                        side[7] += [Ap]
                        side[8] += [Bp(g) for g in GO]
                        spread(Cp(2) + Cp(0) + Cp(1), [8])
                    if doD:
                        spread(Dp(2) + Dp(0) + Dp(1), [9])
                        side[9] += [Ep(g) for g in GO]
                        side[10] += [E2p]
                elif plan == 5:
                    if doA:
                        side[6] += [Ap]
                        side[7] += [Bp(g) for g in GO]
                        spread(Cp(2) + Cp(0) + Cp(1), [8])
                    if doD:
                        spread(Dp(2) + Dp(0) + Dp(1), [8, 9])
                        side[9] += [Ep(g) for g in GO]
                        side[10] += [E2p]
                elif plan == 6:
                    if doD:
                        spread(Dp(2) + Dp(0) + Dp(1), [6])
                        side[7] += [Ep(g) for g in GO]
                        side[8] += [E2p]
                    if doA:
                        side[7] += [Ap]
                        side[9] += [Bp(g) for g in GO]
                        spread(Cp(2) + Cp(0) + Cp(1), [9, 10])
                elif plan == 3:
                    if doD:
                        spread(Dp(2) + Dp(0) + Dp(1), [0, 1, 2])
                        side[3] += [Ep(g) for g in GO]
                        side[4] += [E2p]
                    if doA:
                        side[6] += [Ap]
                        for i_, g in enumerate(GO):
                            side[7 + i_] += [Bp(g)]
                            side[8 + i_] += Cp(g)
                for j in range(7):
                    M1_piece(sl, j)
                    for f in side[j]: f()
                for t in range(5):
                    M2_piece(c, t, last)
                    for f in side[7 + t]: f()
                if last: out_start(c)
            if not last:
                fwd_all(NCH - 1)

        if only is not None:
            fd_cp.wait(); wait(xcopies)
            for l in wpieces + gpieces: start(l)
            start([fi_cp, w1_cp, w2_cp])
            for l in wpieces + gpieces: wait(l)
            wait([fi_cp, w1_cp, w2_cp])
            with jax.named_scope("R"):
                row_phase(only == 'R2')
            if only != 'R2':
                for c in range(NCH):
                    t_ = res[c] + b16(ubuf[pl.ds(128 * c, 128), :]).astype(f32)
                    obuf[c] = t_.astype(bf16).reshape(NS, CH, D); out_start(c)
            for c in range(NCH if only != 'R2' else nch):
                pltpu.make_async_copy(obuf.at[c], o_hbm.at[:, c], sem_o.at[c]).wait()
            return
        def X_piece(c):
            x = xbuf[c].reshape(RC, D).astype(f32)
            A_piece(c, 0, RC, src=x)
        def C_all(c, ab):
            CH_piece(c, ab)
            for g in (0, 1):
                for s0 in range(4): C1_piece(g, s0, ab)
                for k1 in range(4): C2_piece(c, g, k1)
        AB = [abuf, abuf2]
        DM = {'w0': wpieces[0], 'w1': wpieces[1], 'w2': wpieces[2], 'w3': wpieces[3], 'fd': [fd_cp],
              'fi': [fi_cp], 'm1': [w1_cp], 'm2': [w2_cp]}
        for i_ in range(4): DM[f'g{i_}'] = gpieces[i_]
        for c in range(NCH): DM[f'x{c}'] = [xcopies[c]]
        for si, region in enumerate(R0PROG.split('|')):
          with jax.named_scope(f"R0_{si}"):
            for tok in region.split():
                if tok[0] == '>': start(DM[tok[1:]])
                elif tok[0] == '?': wait(DM[tok[1:]])
                elif tok[0] == 'X': X_piece(int(tok[1:]))
                elif tok[0] == 'B':
                    c = int(tok[1:])
                    for g in GO: B_piece(c, g, AB[c % 2])
                elif tok[0] == 'C': C_all(int(tok[1:]), AB[int(tok[1:]) % 2])
                elif tok[0] == 'W':
                    for j in range(int(tok[1:]), int(tok[1:]) + 1): wfix(j); wprep(j)
                else: raise ValueError(tok)
        with jax.named_scope("C1"):
            col_phase(True)
        wait([fi_cp, w1_cp, w2_cp])
        if stop == 1:
            for c in range(NCH):
                inv_all(c, None)
                obuf[c] = res[c].astype(bf16).reshape(NS, CH, D); out_start(c)
        else:
            with jax.named_scope("R1"):
                row_phase(False)
            if stop == 2:
                for c in range(NCH):
                    t_ = res[c] + b16(ubuf[pl.ds(128 * c, 128), :]).astype(f32)
                    obuf[c] = t_.astype(bf16).reshape(NS, CH, D); out_start(c)
            else:
                with jax.named_scope("C2"):
                    col_phase(False)
                with jax.named_scope("R2"):
                    row_phase(True)
        for c in range(NCH):
            pltpu.make_async_copy(obuf.at[c], o_hbm.at[:, c], sem_o.at[c]).wait()

    def fn(A_x, A_w_r, A_w_i, B_x, B_w1, B_b1, B_w2, B_b2):
        hbm = pl.BlockSpec(memory_space=pltpu.HBM)
        vm = pl.BlockSpec(memory_space=pltpu.VMEM)
        dsh = (128, D)
        out = pl.pallas_call(
            kern, out_shape=jax.ShapeDtypeStruct((NS, NCH, CH, D), bf16),
            in_specs=[hbm, hbm, hbm, hbm, vm, hbm, vm, hbm, hbm, hbm, hbm],
            out_specs=hbm,
            scratch_shapes=[
                pltpu.VMEM((NCH, NS, CH, D), bf16),
                pltpu.VMEM((NCH, RC, D), f32),
                pltpu.VMEM((DF, S), bf16), pltpu.VMEM((DF, S), bf16),
                pltpu.VMEM((2, 16, DF, 128), f32),
                pltpu.VMEM((F, D), bf16), pltpu.VMEM((F, D), bf16),
                pltpu.VMEM(dsh, u32), pltpu.VMEM(dsh, u32),
                pltpu.VMEM((NS, 128, 128), u32), pltpu.VMEM((NS, 128, 128), u32),
                pltpu.VMEM((NS, NL, 768), f32),
                pltpu.VMEM((NS * NL // 2, D), u32),
                pltpu.VMEM((NS, NL, D), f32),
                pltpu.VMEM((NCH, NS, CH, D), bf16),
                pltpu.VMEM((RC, D), u32),
                pltpu.VMEM((RC // 2, F), u32),
                pltpu.VMEM((RC, D), u32),
                pltpu.VMEM((RC, D), f32),
                pltpu.VMEM((RC, D), f32),
                pltpu.VMEM((RC // 2, D), u32),
                pltpu.VMEM((RC, D), f32),
                pltpu.VMEM((RC, D), f32),
                pltpu.SemaphoreType.DMA((NCH,)), pltpu.SemaphoreType.DMA((8,)), pltpu.SemaphoreType.DMA((NCH,)), pltpu.SemaphoreType.DMA((8,)), pltpu.SemaphoreType.DMA((4,)),
            ],
            compiler_params=pltpu.CompilerParams(vmem_limit_bytes=100 * 1024 * 1024, flags=flags),
        )(A_x.reshape(NS, NCH, CH, D), A_w_r.T, A_w_i.T, B_w1.T, B_b1, B_w2, B_b2, *consts)
        return out.reshape(1, S, D)
    return fn


_impl = make(**{'plan':4,'prog':0})


@jax.jit
def pallas_interleave_layers__spectral_gfnet__dense_activation_gelu__prompt_kernel(
    A_x: jax.Array,
    A_w_r: jax.Array,
    A_w_i: jax.Array,
    B_x: jax.Array,
    B_w1: jax.Array,
    B_b1: jax.Array,
    B_w2: jax.Array,
    B_b2: jax.Array,
):
    return _impl(A_x, A_w_r, A_w_i, B_x, B_w1, B_b1, B_w2, B_b2)
```

```python
import numpy as np
import jax
import jax.numpy as jnp
from jax import lax
from jax.experimental import pallas as pl
from jax.experimental.pallas import tpu as pltpu

S, D, F, DF = 2048, 640, 1728, 321
NS, NL = 16, 128
CH = 16
NCH = NL // CH
RC = NS * CH
NT = (((1,), (1,)), ((), ()))
f32, bf16, u32 = jnp.float32, jnp.bfloat16, jnp.uint32
R2 = float(np.sqrt(0.5))
C1, C2 = float(np.cos(2 * np.pi / 5)), float(np.cos(4 * np.pi / 5))
S1, S2 = float(np.sin(2 * np.pi / 5)), float(np.sin(4 * np.pi / 5))
KQ = (C1 - C2) / 2
M1E = [0, 256, 512, 768, 1024, 1280, 1536, F]


def p32(x):
    return pltpu.bitcast(x, u32)


def b16(x):
    return pltpu.bitcast(x, bf16)


def _constants():
    j64 = 5 * np.arange(64)
    LA = np.concatenate([1 + j64, 4 + j64])
    LB = np.concatenate([2 + j64, 3 + j64])
    LH = 5 + j64
    d2 = np.arange(128)

    def angle(rows, cols):
        return 2 * np.pi * (np.outer(rows, cols) % D) / D

    def fwd_mat(L, c, iscale):
        th = angle(d2, L)
        sg = np.where(L % 5 == c, 1.0, -1.0)[None, :]
        top = np.concatenate([np.cos(th), -np.sin(th)], axis=1)
        bot = np.concatenate([sg * np.sin(th), sg * np.cos(th)], axis=1) * iscale
        return np.concatenate([top, bot], axis=0)

    th = angle(d2, LH)
    MH = np.concatenate([np.cos(th), -np.sin(th)], axis=1)
    th = angle(LH, d2)
    cw = (np.where(LH == 320, 1.0, 2.0) / (S * D))[:, None]
    NH = np.concatenate([np.cos(th) * cw, -np.sin(th) * cw], axis=0)

    fm = np.zeros((256, 640))
    fm[:, 0:256] = fwd_mat(LA, 1, -S1)
    fm[:, 256:512] = fwd_mat(LB, 2, -S2)
    fm[:128, 512:640] = MH

    fg = np.zeros((128, 896))
    ig = np.zeros((128, 896))
    for q, (L, c, beta) in enumerate(((LA, 1, -S1), (LB, 2, -S2))):
        th = angle(d2, L)
        sg = np.where(L % 5 == c, 1.0, -1.0)[None, :]
        fg[:, 384 * q:384 * q + 128] = np.cos(th)
        fg[:, 384 * q + 128:384 * q + 256] = sg * beta * np.sin(th)
        fg[:, 384 * q + 256:384 * q + 384] = -np.sin(th) + sg * beta * np.cos(th)
        tt = (sg * th).T
        cw = 2.0 / (S * D)
        ig[:, 384 * q:384 * q + 128] = cw * np.cos(tt)
        ig[:, 384 * q + 128:384 * q + 256] = -cw * np.sin(tt)
        ig[:, 384 * q + 256:384 * q + 384] = cw * (np.sin(tt) + np.cos(tt))
    fg[:, 768:896] = MH
    ig[:, 768:896] = NH

    kap = (np.arange(NS)[:, None] + 16 * np.arange(2)[None, :]).reshape(-1)[:, None, None]
    kc = np.arange(64)[None, :, None]
    sp = np.arange(64)[None, None, :]
    g = np.exp(-2j * np.pi * ((sp * (kap + 32 * kc)) % S) / S)

    def realform(m):
        o = np.zeros((32, 128, 128))
        o[:, 0:64, 0::2] = m.real
        o[:, 0:64, 1::2] = -m.imag
        o[:, 64:128, 0::2] = m.imag
        o[:, 64:128, 1::2] = m.real
        return o

    gf = realform(g)
    gi = realform(np.conj(np.transpose(g, (0, 2, 1))))

    def pack(a):
        a = np.asarray(a.astype(jnp.bfloat16)).view(np.uint16).astype(np.uint32)
        return a[..., 0::2, :] | (a[..., 1::2, :] << 16)

    return [pack(fm), pack(ig), pack(gf), pack(gi), pack(fg)]


_CONSTS = _constants()


def layernorm(x):
    m = jnp.mean(x, axis=-1, keepdims=True)
    xc = x - m
    v = jnp.mean(xc * xc, axis=-1, keepdims=True)
    return xc * lax.rsqrt(v + 1e-5)


def gelu(h):
    c = float(np.sqrt(2 / np.pi))
    t = jnp.tanh(h * (c + (0.044715 * c) * (h * h)))
    hh = 0.5 * h
    return hh + hh * t


def tiles(x):
    return [x[:, 128 * t:128 * (t + 1)] for t in range(x.shape[1] // 128)]


class Pair:
    def __init__(s, re, im):
        s.re, s.im = re, im

    def rows(s, a, b):
        return Pair(s.re[a:b], s.im[a:b])

    def cat(s, o):
        return Pair(jnp.concatenate([s.re, o.re], axis=0), jnp.concatenate([s.im, o.im], axis=0))

    def __add__(s, o):
        return Pair(s.re + o.re, s.im + o.im)

    def __sub__(s, o):
        return Pair(s.re - o.re, s.im - o.im)

    def add_i(s, o, sign):
        return Pair(s.re - o.im, s.im + o.re) if sign > 0 else Pair(s.re + o.im, s.im - o.re)

    def tw(s, num, sign):
        num = num % 32
        if num == 0:
            return s
        c = float(np.cos(2 * np.pi * num / 32))
        sn = sign * float(np.sin(2 * np.pi * num / 32))
        if num % 8 == 0:
            q = num // 8
            if q == 2:
                return Pair(-s.re, -s.im)
            sg = sign if q == 1 else -sign
            return Pair(-s.im, s.re) if sg > 0 else Pair(s.im, -s.re)
        if num % 4 == 0:
            if sn * c > 0:
                return Pair((s.re - s.im) * c, (s.re + s.im) * c)
            return Pair((s.re + s.im) * c, (s.im - s.re) * c)
        return Pair(s.re * c - s.im * sn, s.re * sn + s.im * c)


class Half:
    def __init__(s, h, sgn):
        s.h, s.sgn = h, sgn

    def cat(s, o):
        return Half(jnp.concatenate([s.h, o.h], axis=0), s.sgn)

    def __add__(s, o):
        return Half(s.h + o.h, s.sgn)

    def __sub__(s, o):
        return Half(s.h - o.h, s.sgn)

    def tw(s, num, sign):
        num = num % 32
        if num == 0:
            return s
        c = float(np.cos(2 * np.pi * num / 32))
        sn = sign * float(np.sin(2 * np.pi * num / 32))
        if num % 8 == 0:
            q = num // 8
            if q == 2:
                return Half(-s.h, s.sgn)
            sg = sign if q == 1 else -sign
            return Half(pltpu.roll(s.h, 64, 1) * (s.sgn * (-sg)), s.sgn)
        return Half(s.h * c + pltpu.roll(s.h, 64, 1) * (s.sgn * (-sn)), s.sgn)


def radix4(x, sign):
    a = x[0] + x[2]
    b = x[0] - x[2]
    c = x[1] + x[3]
    d = x[1] - x[3]
    return [a + c, b.add_i(d, sign), a - c, b.add_i(d, -sign)]


def rdft8(b):
    t0 = b[0] + b[4]; t1 = b[0] - b[4]; t2 = b[2] + b[6]; t3 = b[2] - b[6]
    t4 = b[1] + b[5]; t5 = b[1] - b[5]; t6 = b[3] + b[7]; t7 = b[3] - b[7]
    s02 = t0 + t2; s46 = t4 + t6
    u = (t5 - t7) * R2; v = (t5 + t7) * R2
    return [s02 + s46, t1 + u, t0 - t2, t1 - u, s02 - s46], [None, t3 + v, t4 - t6, v - t3, None]


def rdft16(a):
    Ec, Es = rdft8(a[0::2])
    Oc, Os = rdft8(a[1::2])
    C = [None] * 9
    Sn = [None] * 8
    C[0] = Ec[0] + Oc[0]; C[8] = Ec[0] - Oc[0]; C[4] = Ec[4]; Sn[4] = Oc[4]
    for k in (1, 2, 3):
        c = float(np.cos(2 * np.pi * k / 16))
        s = float(np.sin(2 * np.pi * k / 16))
        if k == 2:
            P = (Oc[k] - Os[k]) * R2
            Q = (Os[k] + Oc[k]) * R2
        else:
            P = c * Oc[k] - s * Os[k]
            Q = c * Os[k] + s * Oc[k]
        C[k] = Ec[k] + P; C[8 - k] = Ec[k] - P
        Sn[k] = Es[k] + Q; Sn[8 - k] = Q - Es[k]
    return C, Sn


def dft16_half(a, sign, sgn):
    Ch, Sh = rdft16(a)
    out = [None] * 16
    out[0] = Ch[0]
    out[8] = Ch[8]
    for k in range(1, 8):
        t = pltpu.roll(Sh[k], 64, 1) * sgn
        if sign < 0:
            out[k] = Ch[k] + t; out[16 - k] = Ch[k] - t
        else:
            out[k] = Ch[k] - t; out[16 - k] = Ch[k] + t
    return out


GRP = [(0, 1), (2, 3)]
GO = (2, 0, 1)

PLAN1 = dict(A=0, B=2, C=2, D=7, E=8, E2=8, nA=4, nE=2, chain="CDEA", gate_c=6, barrier=(3,))
PLAN2 = dict(A=0, B=2, C=3, D=7, E=8, E2=9, nA=1, nE=4, chain="DE", gate_c=None, barrier=())


def _kernel(x_hbm, wrt_hbm, wit_hbm, w1t_hbm, b1_ref, w2_hbm, b2_ref, fd_hbm, fi_hbm, gf_hbm, gi_hbm, fg_hbm,
            o_hbm,
            xbuf, res, wrt, wit, wtf, w1t, w2, fd, fi, fg, ub7, w1s, w2s, b1c, gf, gi, wpp, ubuf, vbuf, obuf,
            xnb, gbuf, ub, abuf, tbuf, zbuf, abuf2, tbuf2,
            sem_x, sem_w, sem_o, sem_g, sem_m, sem_b, sem_t):
    xcp = [pltpu.make_async_copy(x_hbm.at[:, :, c], xbuf.at[c], sem_x.at[c]) for c in range(NCH)]
    wsl = lambda j: pl.ds(512 * j, 512)
    wcp = [[pltpu.make_async_copy(h.at[:, wsl(j)], v.at[:, wsl(j)], sem_w.at[2 * j + i])
            for i, (h, v) in enumerate(((wrt_hbm, wrt), (wit_hbm, wit)))] for j in range(4)]
    gcp = [[pltpu.make_async_copy(h.at[pl.ds(8 * j, 8)], v.at[pl.ds(8 * j, 8)], sem_g.at[2 * j + i])
            for i, (h, v) in enumerate(((gf_hbm, gf), (gi_hbm, gi)))] for j in range(4)]
    fd_cp = [pltpu.make_async_copy(fd_hbm, fd, sem_m.at[0])]
    fi_cp = [pltpu.make_async_copy(fi_hbm, fi, sem_m.at[1]), pltpu.make_async_copy(fg_hbm, fg, sem_m.at[4])]
    w1_cp = [pltpu.make_async_copy(w1t_hbm, w1t, sem_m.at[2])]
    w2_cp = [pltpu.make_async_copy(w2_hbm, w2, sem_m.at[3])]

    def start(l):
        for cp in l:
            cp.start()

    def wait(l):
        for cp in l:
            cp.wait()

    def out_cp(c):
        return pltpu.make_async_copy(obuf.at[c], o_hbm.at[:, :, c], sem_o.at[c])

    def tail_cp(t):
        lanes = pl.ds(128 * t, 128)
        return pltpu.make_async_copy(obuf.at[NCH - 1, :, :, :, lanes], o_hbm.at[:, :, NCH - 1, :, lanes], sem_t.at[t])

    lane = lax.broadcasted_iota(jnp.int32, (1, 128), 1)
    sgn = jnp.where(lane < 64, 1.0, -1.0).astype(f32)

    def rs(s, n=CH):
        return pl.ds(n * s, n)

    def ld(ref, idx, grp):
        return Pair(ref[idx + (pl.ds(128 * grp[0], 128),)], ref[idx + (pl.ds(128 * grp[1], 128),)])

    def st(ref, idx, grp, val):
        ref[idx + (pl.ds(128 * grp[0], 128),)] = val.re
        ref[idx + (pl.ds(128 * grp[1], 128),)] = val.im

    state = dict(chain="", C=None, D=None, A=None, E=None)

    def always():
        return fd[120:128, 512:640] == 0

    def gate(name, a):
        dep = state[name]
        if dep is None:
            return a
        n = a.shape[0] // 8
        m = always()
        if n > 1:
            m = jnp.concatenate([m] * n, axis=0)
            dep = jnp.concatenate([dep] * n, axis=0)
        return jnp.where(m, a, dep)

    def gate2(name, v):
        return Pair(gate(name, v.re), gate(name, v.im))

    def mark(name, arr):
        state[name] = pltpu.roll(arr[0:8], 1, 1) if name in state["chain"] else None

    def radix5_fwd(x):
        x0, x1, x2, x3, x4 = tiles(layernorm(x))
        t1 = x1 + x4; t2 = x2 + x3; t3 = x1 - x4; t4 = x2 - x3
        p = t1 + t2
        q = (t1 - t2) * KQ
        u0 = x0 + p
        m = x0 - 0.25 * p
        return m + q, t3 + (S2 / S1) * t4, m - q, t3 - (S1 / S2) * t4, u0

    def a_piece(c, r0, nr):
        x = res[c, pl.ds(r0, nr), :]
        x = jnp.concatenate([gate("A", x[:, 0:128]), x[:, 128:]], axis=1)
        u1r, u1i, u2r, u2i, u0 = radix5_fwd(x)
        u = jnp.concatenate([u1r, u1i, u1r + u1i, u2r, u2i, u2r + u2i, u0], axis=1)
        ub7[pl.ds((c % 2) * (RC // 2) + r0 // 2, nr // 2), :] = p32(u.astype(bf16))
        mark("A", u0)

    def b_piece(c, g):
        def dot(o):
            lhs = b16(ub7[pl.ds((c % 2) * (RC // 2), RC // 2), o:o + 128])
            return jnp.dot(lhs, b16(fg[:, o:o + 128]), preferred_element_type=f32)
        if g == 2:
            abuf[:, 512:640] = dot(768)
            return
        beta = (-S1, -S2)[g]
        p1 = dot(384 * g); p2 = dot(384 * g + 128); p3 = dot(384 * g + 256)
        abuf[:, 256 * g:256 * g + 128] = p1 + p2
        abuf[:, 256 * g + 128:256 * g + 256] = p3 + (sgn * (-beta)) * p1 + (sgn * (1.0 / beta)) * p2

    def x_piece(c):
        for i in range(4):
            x = xbuf[c, pl.ds(4 * i, 4)].astype(f32).reshape(64, D)
            u = jnp.concatenate(radix5_fwd(x), axis=1)
            ub[pl.ds(c * (RC // 2) + 32 * i, 32), :] = p32(u.astype(bf16))

    def b0_piece(c, g):
        lo = (0, 256, 512)[g]
        w = (256, 256, 128)[g]
        lhs = b16(ub[pl.ds(c * (RC // 2), RC // 2), lo:lo + w])
        res[c, :, lo:lo + w] = jnp.dot(lhs, b16(fd[0:w // 2, lo:lo + w]), preferred_element_type=f32)

    def c1_piece(ab, g, s0):
        grp = GRP[g]
        x = [ld(ab, (rs(4 * s1 + s0),), grp) for s1 in range(4)]
        x[0] = gate2("C", x[0])
        y = radix4(x, -1)
        for k1 in range(4):
            o = y[k1].tw(2 * k1 * s0, -1)
            st(tbuf, (rs(4 * s0 + k1),), grp, o)
        mark("C", o.im[8:16])

    def c2_piece(c, g, k1):
        grp = GRP[g]
        x = [ld(tbuf, (rs(4 * s0 + k1),), grp) for s0 in range(4)]
        x[0] = gate2("C", x[0])
        y = radix4(x, -1)
        for k2 in range(4):
            ka = k1 + 4 * k2
            u0 = y[k2].rows(0, 8)
            u1 = y[k2].rows(8, 16).tw(ka, -1)
            for p, bp in enumerate((u0 + u1, u0 - u1)):
                ubuf[pl.ds(64 * ka + 8 * c, 8), pl.ds(256 * p + 128 * g, 128)] = (
                    pltpu.pack_elementwise([bp.re, bp.im], packed_dtype=bf16))
        mark("C", bp.im)

    def ch_piece(ab, c):
        y = dft16_half([ab[rs(s), 512:640] for s in range(NS)], -1, sgn)
        for k in range(NS):
            u0 = Half(y[k][0:8], sgn)
            u1 = Half(y[k][8:16], sgn).tw(k, -1)
            ubuf[pl.ds(64 * k + 8 * c, 8), 512:640] = (
                pltpu.pack_elementwise([(u0 + u1).h, (u0 - u1).h], packed_dtype=bf16))

    def c_group(ab, c, g):
        if g == 2:
            ch_piece(ab, c)
            return
        for s0 in range(4):
            c1_piece(ab, g, s0)
        for k1 in range(4):
            c2_piece(c, g, k1)

    def dh_piece(c):
        x = []
        for k in range(NS):
            v0 = Half(vbuf[k, pl.ds(8 * c, 8), 512:640], sgn)
            v1 = Half(vbuf[k, pl.ds(8 * c, 8), D + 512:2 * D], sgn)
            x.append((v0 + v1).cat((v0 - v1).tw(k, 1)).h)
        y = dft16_half(x, 1, sgn)
        for s in range(NS):
            zbuf[rs(s, CH // 2), 768:896] = p32(y[s].astype(bf16))

    def d1_piece(c, g, k0):
        grp = GRP[g]
        x = []
        for k1 in range(4):
            ka = 4 * k1 + k0
            v0 = ld(vbuf, (ka, pl.ds(8 * c, 8)), grp)
            v1 = ld(vbuf, (ka, pl.ds(8 * c, 8)), (grp[0] + 5, grp[1] + 5))
            if k1 == 0:
                v0 = gate2("D", v0)
            x.append((v0 + v1).cat((v0 - v1).tw(ka, 1)))
        y = radix4(x, 1)
        for s1 in range(4):
            o = y[s1].tw(2 * s1 * k0, 1)
            st(tbuf2, (rs(4 * k0 + s1),), grp, o)
        mark("D", o.im[8:16])

    def d2_piece(g, s1):
        grp = GRP[g]
        x = [ld(tbuf2, (rs(4 * k0 + s1),), grp) for k0 in range(4)]
        x[0] = gate2("D", x[0])
        y = radix4(x, 1)
        for s2 in range(4):
            zi = y[s2].im * sgn
            z = jnp.concatenate([y[s2].re, zi, y[s2].re + zi], axis=1)
            zbuf[rs(s1 + 4 * s2, CH // 2), 384 * g:384 * g + 384] = p32(z.astype(bf16))
        mark("D", y[3].im[8:16])

    def d_group(c, g, stage1=True):
        if g == 2:
            dh_piece(c)
            return
        if stage1:
            for k0 in range(4):
                d1_piece(c, g, k0)
        for s1 in range(4):
            d2_piece(g, s1)

    def e_piece(g):
        def dot(o):
            return jnp.dot(b16(zbuf[:, o:o + 128]), b16(fi[:, o:o + 128]), preferred_element_type=f32)
        if g == 2:
            abuf2[:, 512:640] = dot(768)
            return
        p1 = dot(384 * g); p2 = dot(384 * g + 128); p3 = dot(384 * g + 256)
        abuf2[:, 256 * g:256 * g + 128] = p1 + p2
        abuf2[:, 256 * g + 128:256 * g + 256] = p3 - p1 + p2

    def e2_piece(c, r0, nr, first):
        v1r, a1, v2r, a2, v0 = tiles(abuf2[pl.ds(r0, nr), :])
        v1r = gate("E", v1r)
        t1 = v1r + v2r
        n = (v1r - v2r) * KQ
        y0 = v0 + t1
        m = v0 - 0.25 * t1
        aa = m + n
        bb = m - n
        p = S1 * a1 + S2 * a2
        q = S2 * a1 - S1 * a2
        y = jnp.concatenate([y0, aa - p, bb - q, bb + q, aa + p], axis=1)
        if first:
            x0 = xbuf[c, pl.ds(r0 // 16, nr // 16)].astype(f32).reshape(nr, D)
        else:
            x0 = res[c, pl.ds(r0, nr), :]
        x1 = x0 + y
        res[c, pl.ds(r0, nr), :] = x1
        xn = layernorm(x1)
        xnb[pl.ds((c % 2) * (RC // 2) + r0 // 2, nr // 2), :] = p32(xn.astype(bf16))
        mark("E", xn[:, 0:128])

    def m1_piece(c, j, dep):
        a, b = M1E[j], M1E[j + 1]
        bias = b1c[a:b, :]
        if dep is not None:
            bias = jnp.concatenate([jnp.where(always()[0:1], bias[0:8], dep), bias[8:]], axis=0)
        bias = jnp.concatenate([bias] * (RC // 128), axis=1)
        xn = b16(xnb[pl.ds((c % 2) * (RC // 2), RC // 2), :])
        ht = lax.dot_general(b16(w1s[a // 2:b // 2, :]), xn, NT, preferred_element_type=f32) + bias
        gbuf[:, a:b] = p32(gelu(ht).astype(bf16).T)

    def m2_piece(c, t, last):
        a, b = 128 * t, 128 * (t + 1)
        o = jnp.dot(b16(gbuf[...]), b16(w2s[:, a:b]), preferred_element_type=f32)
        o = o + b2_ref[...].astype(f32).reshape(1, D)[:, a:b]
        x2 = res[c, :, a:b] + o
        if last:
            obuf[c, :, :, :, a:b] = x2.reshape(NS, 2, 8, 128).astype(bf16)
            if c == NCH - 1:
                tail_cp(t).start()
        else:
            res[c, :, a:b] = x2

    rr = lax.broadcasted_iota(jnp.int32, (128, 128), 0)
    cc = lax.broadcasted_iota(jnp.int32, (128, 128), 1)
    pm = jnp.where((rr // 8) + 16 * (rr % 8) == cc, 1.0, 0.0).astype(bf16)

    def w_piece(j):
        wtf[0, j] = wrt[:, pl.ds(128 * j, 128)].astype(f32)
        wtf[1, j] = wit[:, pl.ds(128 * j, 128)].astype(f32)

        def rows(i, c0, c1):
            r = [wtf[i, j, pl.ds(c0, 64, stride=5), :], wtf[i, j, pl.ds(c1, 64, stride=5), :]]
            return jnp.concatenate(r, axis=0).astype(bf16)
        rhs = [rows(0, 1, 4), rows(1, 1, 4), rows(0, 2, 3), rows(1, 2, 3), rows(0, 5, 5), rows(1, 5, 5)]
        outs = [lax.dot_general(pm, r, NT, preferred_element_type=f32) for r in rhs]
        outs[5] = outs[5] * (-sgn)
        for t in range(3):
            pk = pltpu.pack_elementwise([outs[2 * t], outs[2 * t + 1]], packed_dtype=bf16)
            for ka in range(NS):
                wpp[ka, t, pl.ds(8 * j, 8), :] = pk[8 * ka:8 * (ka + 1)]

    even = (lane % 2) == 0

    def two_stage(l0, l1, r):
        z = jnp.zeros_like(l0)
        a = jnp.where(even, l0, z)
        b = jnp.where(even, z, l1)
        x0 = jnp.dot(b16(l0), b16(r[:, 0:256]), preferred_element_type=f32)
        x1 = jnp.dot(b16(l1), b16(r[:, 256:512]), preferred_element_type=f32)
        lh = b16(jnp.concatenate([a, b[32:64], b[0:32]], axis=0))
        xh = jnp.dot(lh, b16(r[:, 512:640]), preferred_element_type=f32)
        xh0 = xh[0:64] - pltpu.roll(xh[64:128], 64, 1) * sgn
        xh1 = xh[128:192] + pltpu.roll(xh[192:256], 64, 1) * sgn
        return x0, x1, xh0, xh1

    def col_a(ka):
        return two_stage(gf[2 * ka], gf[2 * ka + 1], ubuf[pl.ds(64 * ka, 64), :])

    def col_b(ka, xs):
        outs = []
        yh = []
        for p in range(2):
            w = []
            for t in range(3):
                pk = wpp[ka, t, pl.ds(p, 64, stride=2), :]
                w += [pltpu.unpack_elementwise(pk, index=i, packed_dtype=bf16, unpacked_dtype=f32) for i in range(2)]
            for q in range(2):
                xr = xs[p][0:64, 128 * q:128 * (q + 1)]
                xi = xs[p][64:128, 128 * q:128 * (q + 1)]
                wr, wi = w[2 * q], w[2 * q + 1]
                outs.append(pltpu.pack_elementwise([xr * wr - xi * wi, xr * wi + xi * wr], packed_dtype=bf16))
            xh = xs[2 + p]
            yh.append(xh * w[4] + pltpu.roll(xh, 64, 1) * w[5])
        outs.append(pltpu.pack_elementwise(yh, packed_dtype=bf16))
        return jnp.concatenate(outs, axis=1)

    def col_c(ka, yb):
        v0, v1, vh0, vh1 = two_stage(gi[2 * ka], gi[2 * ka + 1], yb)
        for p, (v, vh) in enumerate(((v0, vh0), (v1, vh1))):
            o = D * p
            vbuf[ka, :, o:o + 128] = v[0:64, 0:128]
            vbuf[ka, :, o + 128:o + 256] = v[64:128, 0:128]
            vbuf[ka, :, o + 256:o + 384] = v[0:64, 128:256]
            vbuf[ka, :, o + 384:o + 512] = v[64:128, 128:256]
            vbuf[ka, :, o + 512:o + 640] = vh

    def col_phase():
        order = [4 * (i % 4) + i // 4 for i in range(NS)]
        q = [col_a(order[i]) for i in range(3)]
        for i in range(NS):
            if i + 3 < NS:
                q.append(col_a(order[i + 3]))
            col_c(order[i], col_b(order[i], q.pop(0)))
            if (i + 1) % 4 == 0:
                for g in (0, 1):
                    d1_piece(0, g, i // 4)

    def row_phase(last):
        plan = PLAN2 if last else PLAN1
        first = not last
        state.update(chain="", C=None, D=None, A=None, E=None)
        for g in GO:
            d_group(0, g, stage1=False)
        for g in GO:
            e_piece(g)
        e2_piece(0, 0, RC, first)
        for c in range(NCH):
            state.update(chain=plan["chain"], C=None, D=None, A=None, E=None)
            do_a = first and c > 0
            do_d = c + 1 < NCH

            def d_start():
                state["D"] = pltpu.bitcast(gbuf[0:8, 1536:1664], f32)

            def all_a():
                n = plan["nA"]
                for i in range(n):
                    a_piece(c - 1, i * (RC // n), RC // n)

            def all_e2():
                n = plan["nE"]
                for i in range(n):
                    e2_piece(c + 1, i * (RC // n), RC // n, first)

            work = []
            if do_a:
                work += [(plan["A"], 0, all_a),
                         (plan["B"], 1, lambda: [b_piece(c - 1, g) for g in GO]),
                         (plan["C"], 2, lambda: [c_group(abuf, c - 1, g) for g in GO])]
            if do_d:
                work += [(plan["D"], 3, lambda: [d_group(c + 1, g) for g in GO]),
                         (plan["E"], 4, lambda: [e_piece(g) for g in GO]),
                         (plan["E2"], 5, all_e2)]
            side = {i: [] for i in range(12)}
            side[6].append(d_start)
            for slot, _, fn in sorted(work, key=lambda t: t[:2]):
                side[slot].append(fn)

            convert = first and c == 0
            for j in range(7):
                if convert:
                    w1s[M1E[j] // 2:M1E[j + 1] // 2, :] = p32(w1t[M1E[j]:M1E[j + 1], :])
                dep = None
                if do_a and plan["gate_c"] == j:
                    acc = None
                    for r0, c0 in [(64 * k, l) for k in (12, 13, 14, 15) for l in (128, 384)] + [(64 * 15, 512)]:
                        v = ubuf[pl.ds(r0 + 8 * (c - 1), 8), pl.ds(c0, 128)]
                        acc = v if acc is None else acc | v
                    dep = pltpu.bitcast(acc, f32)
                m1_piece(c, j, dep)
                for fn in side[j]:
                    fn()
            if convert:
                wait(w2_cp)
            for t in range(5):
                if convert:
                    w2s[:, 128 * t:128 * (t + 1)] = p32(w2[:, 128 * t:128 * (t + 1)])
                m2_piece(c, t, last)
                for fn in side[7 + t]:
                    fn()
            if last and c < NCH - 1:
                out_cp(c).start()
            if c in plan["barrier"]:
                pl.semaphore_signal(sem_b, 1)
                pl.semaphore_wait(sem_b, 1)
        if first:
            state.update(chain="", C=None, D=None, A=None, E=None)
            a_piece(NCH - 1, 0, RC)
            for g in GO:
                b_piece(NCH - 1, g)
            for g in GO:
                c_group(abuf, NCH - 1, g)

    def b0(c):
        for g in GO:
            b0_piece(c, g)

    def c0(c):
        for g in GO:
            c_group(res.at[c], c, g)

    def w4(j):
        for i in range(4 * j, 4 * j + 4):
            w_piece(i)

    start(fd_cp + xcp[0:2])
    b1c[...] = jnp.broadcast_to(b1_ref[...].astype(f32).reshape(1, F), (128, F)).T
    wait(fd_cp + xcp[0:1])
    start(xcp[2:8])
    x_piece(0)
    wait(xcp[1:3])
    start(wcp[0])
    b0(0); x_piece(1); b0(1); x_piece(2); c0(0)
    wait(xcp[3:5])
    start(wcp[1] + wcp[2] + wcp[3])
    b0(2); x_piece(3); c0(1); b0(3); x_piece(4); c0(2)
    wait(xcp[5:8] + wcp[0])
    start(gcp[0] + gcp[1] + gcp[2] + gcp[3])
    b0(4); x_piece(5); c0(3); b0(5); x_piece(6); c0(4); w4(0)
    wait(wcp[1] + wcp[2])
    start(fi_cp + w1_cp)
    b0(6); x_piece(7); c0(5); w4(1); b0(7); c0(6); w4(2)
    wait(wcp[3])
    c0(7); w4(3)
    start(w2_cp)

    wait(gcp[0] + gcp[1] + gcp[2] + gcp[3])
    col_phase()
    wait(fi_cp + w1_cp)
    row_phase(False)
    col_phase()
    row_phase(True)
    for c in range(NCH - 1):
        out_cp(c).wait()
    for t in range(5):
        tail_cp(t).wait()


@jax.jit
def pallas_interleave_layers__spectral_gfnet__dense_activation_gelu__prompt_kernel(
    A_x: jax.Array,
    A_w_r: jax.Array,
    A_w_i: jax.Array,
    B_x: jax.Array,
    B_w1: jax.Array,
    B_b1: jax.Array,
    B_w2: jax.Array,
    B_b2: jax.Array,
):
    hbm = pl.BlockSpec(memory_space=pltpu.HBM)
    vm = pl.BlockSpec(memory_space=pltpu.VMEM)
    io_shape = (NS, 2, NCH, 8, D)
    dma = pltpu.SemaphoreType.DMA
    out = pl.pallas_call(
        _kernel,
        out_shape=jax.ShapeDtypeStruct(io_shape, bf16),
        in_specs=[hbm, hbm, hbm, hbm, vm, hbm, vm, hbm, hbm, hbm, hbm, hbm],
        out_specs=hbm,
        scratch_shapes=[
            pltpu.VMEM((NCH, NS, 2, 8, D), bf16),
            pltpu.VMEM((NCH, RC, D), f32),
            pltpu.VMEM((DF, S), bf16), pltpu.VMEM((DF, S), bf16),
            pltpu.VMEM((2, 16, DF, 128), f32),
            pltpu.VMEM((F, D), bf16), pltpu.VMEM((F, D), bf16),
            pltpu.VMEM((128, D), u32), pltpu.VMEM((64, 896), u32),
            pltpu.VMEM((64, 896), u32), pltpu.VMEM((RC, 896), u32),
            pltpu.VMEM((F // 2, D), u32), pltpu.VMEM((F // 2, D), u32),
            pltpu.VMEM((F, 128), f32),
            pltpu.VMEM((2 * NS, 64, 128), u32), pltpu.VMEM((2 * NS, 64, 128), u32),
            pltpu.VMEM((NS, 3, NL, 128), u32),
            pltpu.VMEM((NS * NL // 2, D), u32),
            pltpu.VMEM((NS, 64, 2 * D), f32),
            pltpu.VMEM((NCH, NS, 2, 8, D), bf16),
            pltpu.VMEM((RC, D), u32),
            pltpu.VMEM((RC // 2, F), u32),
            pltpu.VMEM((NCH * RC // 2, D), u32),
            pltpu.VMEM((RC, D), f32), pltpu.VMEM((RC, D), f32),
            pltpu.VMEM((RC // 2, 896), u32),
            pltpu.VMEM((RC, D), f32), pltpu.VMEM((RC, D), f32),
            dma((NCH,)), dma((8,)), dma((NCH,)), dma((8,)), dma((5,)),
            pltpu.SemaphoreType.REGULAR, dma((5,)),
        ],
        compiler_params=pltpu.CompilerParams(vmem_limit_bytes=100 * 1024 * 1024),
    )(A_x.reshape(io_shape), A_w_r.T, A_w_i.T, B_w1.T, B_b1, B_w2, B_b2, *_CONSTS)
    return out.reshape(1, S, D)
```
